```python
import os as _os
_os.environ.setdefault("JAX_PLATFORMS", "cpu")
import jax
import jax.numpy as jnp

def _softmax(x, axis=-1):
    return jax.nn.softmax(x, axis=axis)
def _gelu(x):
    return jax.nn.gelu(x, approximate=True)
def _silu(x):
    return jax.nn.silu(x)
def _sigmoid(x):
    return jax.nn.sigmoid(x)
def _layernorm(x, axis=-1, eps=1e-5):
    m = jnp.mean(x, axis=axis, keepdims=True)
    v = jnp.var(x, axis=axis, keepdims=True)
    return (x - m) / jnp.sqrt(v + eps)
def _scatter_add(tgt, idx, src, axis=0):
    return tgt.at[idx].add(src)
def _segment_sum(src, seg, n):
    return jax.ops.segment_sum(src, seg, n)
class _Rng:
    def __init__(self, key):
        self._k = key
    def _next(self):
        self._k, sub = jax.random.split(self._k)
        return sub
    def normal(self, shape):
        return jax.random.normal(self._next(), shape, dtype=jnp.bfloat16)
    def randint(self, lo, hi, shape):
        return jax.random.randint(self._next(), shape, lo, hi, dtype=jnp.int32)
    def uniform(self, shape, lo=0.0, hi=1.0):
        return jax.random.uniform(self._next(), shape, jnp.bfloat16, lo, hi)
    def permutation(self, n):
        return jax.random.permutation(self._next(), n)


kernel_name = 'standalone__channel_attn_cbam__vision'

def setup_inputs():
    _rng = _Rng(jax.random.key(int.from_bytes(__import__("os").urandom(4), "little")))
    _w = (lambda a: (lambda t: t.astype(jnp.bfloat16) if jnp.issubdtype(t.dtype, jnp.floating) else t)(jnp.asarray(a)))
    H = W = 224
    C = 192
    r = max(C // 4, 1)
    return {
        "x": _w((lambda *s: _rng.normal(s) * 0.2)(1, H, W, C) + (lambda *s: _rng.normal(s) * 0.2)(1, 1, 1, C) * 2.0),
        "w1": _w((lambda *s: _rng.normal(s) * 0.2)(C, r)),
        "w2": _w((lambda *s: _rng.normal(s) * 0.2)(r, C)),
    }

def reference(x, w1, w2):
    B, H, W, C = x.shape
    xf = x.reshape(B, H * W, C)
    gap = jnp.mean(xf, 1)
    gmp = jnp.amax(xf, 1)
    h_a = gap @ w1
    h_a = h_a * (lambda x, dt: x.astype(dt))(h_a > 0, h_a.dtype)
    h_m = gmp @ w1
    h_m = h_m * (lambda x, dt: x.astype(dt))(h_m > 0, h_m.dtype)
    scale = _sigmoid(h_a @ w2 + h_m @ w2)
    return x * scale[:, None, None, :]
```

```python
import functools

import jax
import jax.numpy as jnp
from jax import lax
import jax.experimental.pallas as pl
import jax.experimental.pallas.tpu as pltpu


_GROUP = 7
_CG = 32


def _read_chunks(n_outer):
    sizes = [8, 8, 8, 4, 2, 1]
    assert sum(sizes) == n_outer - 1
    out = []
    a = 0
    for s in sizes:
        out.append((a, s, 0, _GROUP))
        a += s
    out.append((a, 1, 0, 4))
    out.append((a, 1, 4, 2))
    out.append((a, 1, 6, 1))
    return out


def _write_chunks(n_outer, c):
    half = c // 2
    out = []
    first = True
    for b in range(_GROUP):
        for hf in range(2):
            if first:
                for (a0, n) in [(0, 2), (2, 6), (8, n_outer - 8)]:
                    out.append((a0, n, b, hf * half, half))
                first = False
            else:
                out.append((0, n_outer, b, hf * half, half))
    return out


def _kernel(x_hbm, w1t_hbm, w2_hbm, o_hbm,
            xbuf, w1t_v, w2_v, w2t_v, acc_sum, acc_max, scale_v,
            rsem, wsem, psem, *, n_outer, c, w, inv_hw):
    rchunks = _read_chunks(n_outer)
    wchunks = _write_chunks(n_outer, c)

    def rcopy(i):
        a0, na, b0, nb = rchunks[i]
        sl = (pl.ds(a0, na), pl.ds(b0, nb))
        return pltpu.make_async_copy(x_hbm.at[sl], xbuf.at[sl], rsem.at[i])

    def wcopy(i):
        a0, na, b, c0, nc = wchunks[i]
        sl = (pl.ds(a0, na), pl.ds(b, 1), pl.ds(c0, nc))
        return pltpu.make_async_copy(xbuf.at[sl], o_hbm.at[sl], wsem.at[i])

    w1cp = pltpu.make_async_copy(w1t_hbm, w1t_v, psem.at[0])
    w2cp = pltpu.make_async_copy(w2_hbm, w2_v, psem.at[1])

    rcopy(0).start()
    w1cp.start()
    w2cp.start()
    for i in range(1, len(rchunks)):
        rcopy(i).start()

    acc_sum[...] = jnp.zeros(acc_sum.shape, jnp.float32)
    acc_max[...] = jnp.full(acc_max.shape, -jnp.inf, jnp.float32)

    w1cp.wait()
    w2cp.wait()
    w2t_v[...] = w2_v[...].astype(jnp.float32).T.astype(jnp.bfloat16)

    n_groups = c // _CG

    for i, (a0, na, b0, nb) in enumerate(rchunks):
        rcopy(i).wait()

        def group_body(g, carry, a0=a0, na=na, b0=b0, nb=nb):
            c0 = pl.multiple_of(g * _CG, _CG)

            def outer_body(a, sm):
                s, m = sm
                for b in range(b0, b0 + nb):
                    v = xbuf[a, b, pl.ds(c0, _CG), :].astype(jnp.float32)
                    s = s + v
                    m = jnp.maximum(m, v)
                return s, m

            s0 = acc_sum[pl.ds(c0, _CG), :]
            m0 = acc_max[pl.ds(c0, _CG), :]
            s, m = lax.fori_loop(a0, a0 + na, outer_body, (s0, m0))
            acc_sum[pl.ds(c0, _CG), :] = s
            acc_max[pl.ds(c0, _CG), :] = m
            return carry

        lax.fori_loop(0, n_groups, group_body, 0)

    gap = (jnp.sum(acc_sum[...], axis=1, keepdims=True) * inv_hw)
    gmp = jnp.max(acc_max[...], axis=1, keepdims=True)
    pooled = jnp.concatenate(
        [jnp.broadcast_to(gap, (c, 128)), jnp.broadcast_to(gmp, (c, 128))],
        axis=1).astype(jnp.bfloat16)
    hid = jnp.dot(w1t_v[...], pooled, preferred_element_type=jnp.float32)
    hid = hid.astype(jnp.bfloat16).astype(jnp.float32)
    hid = jnp.where(hid > 0, hid, 0.0).astype(jnp.bfloat16)
    logits = jnp.dot(w2t_v[...], hid, preferred_element_type=jnp.float32)
    logits = logits.astype(jnp.bfloat16).astype(jnp.float32)
    z = (logits[:, :128] + logits[:, 128:]).astype(jnp.bfloat16).astype(jnp.float32)
    sc = jax.nn.sigmoid(z).astype(jnp.bfloat16).astype(jnp.float32)
    scale_v[:, 0:128] = sc
    scale_v[:, 128:256] = sc

    for i, (a0, na, b, c0s, nc) in enumerate(wchunks):
        def group_body2(g, carry, a0=a0, na=na, b=b, c0s=c0s):
            c0 = pl.multiple_of(c0s + g * _CG, _CG)
            s = scale_v[pl.ds(c0, _CG), 0:w]

            def outer_body(a, carry2):
                v = xbuf[a, b, pl.ds(c0, _CG), :].astype(jnp.float32)
                xbuf[a, b, pl.ds(c0, _CG), :] = (v * s).astype(jnp.bfloat16)
                return carry2

            lax.fori_loop(a0, a0 + na, outer_body, 0, unroll=2)
            return carry

        lax.fori_loop(0, nc // _CG, group_body2, 0)
        wcopy(i).start()

    for i in range(len(wchunks)):
        wcopy(i).wait()


@jax.jit
def pallas_standalone__channel_attn_cbam__vision_kernel(
    x: jax.Array,
    w1: jax.Array,
    w2: jax.Array,
):
    B, H, W, C = x.shape
    assert B == 1
    r = w1.shape[1]
    n_outer = H // _GROUP
    x4 = jnp.transpose(x, (0, 1, 3, 2)).reshape(n_outer, _GROUP, C, W)
    w1t = w1.T

    n_r = len(_read_chunks(n_outer))
    n_w = len(_write_chunks(n_outer, C))

    kernel = functools.partial(
        _kernel, n_outer=n_outer, c=C, w=W, inv_hw=1.0 / (H * W))

    out4 = pl.pallas_call(
        kernel,
        in_specs=[
            pl.BlockSpec(memory_space=pl.ANY),
            pl.BlockSpec(memory_space=pl.ANY),
            pl.BlockSpec(memory_space=pl.ANY),
        ],
        out_specs=pl.BlockSpec(memory_space=pl.ANY),
        out_shape=jax.ShapeDtypeStruct((n_outer, _GROUP, C, W), x.dtype),
        scratch_shapes=[
            pltpu.VMEM((n_outer, _GROUP, C, W), x.dtype),
            pltpu.VMEM((r, C), w1.dtype),
            pltpu.VMEM((r, C), w2.dtype),
            pltpu.VMEM((C, r), w2.dtype),
            pltpu.VMEM((C, W), jnp.float32),
            pltpu.VMEM((C, W), jnp.float32),
            pltpu.VMEM((C, 256), jnp.float32),
            pltpu.SemaphoreType.DMA((n_r,)),
            pltpu.SemaphoreType.DMA((n_w,)),
            pltpu.SemaphoreType.DMA((2,)),
        ],
        compiler_params=pltpu.CompilerParams(
            vmem_limit_bytes=64 * 1024 * 1024),
    )(x4, w1t, w2)

    return jnp.transpose(out4.reshape(B, H, C, W), (0, 1, 3, 2))
```

```python
import functools

import jax
import jax.numpy as jnp
from jax import lax
import jax.experimental.pallas as pl
import jax.experimental.pallas.tpu as pltpu


_A = 7
_SPLIT = 2
_RK = 16
_DEPTH = 4
_NLATE = 6
_LATE_GROUPS = ((0, 3), (3, 2), (5, 1))
_CG = 32
_WK = 32
_HEAD = ((0, 16), (16, 16))

_F32 = jnp.float32
_BF16 = jnp.bfloat16


def _body(x_hbm, w1t_hbm, w2_hbm, o_hbm,
          xbuf, w1t_v, w2_v, w1e_v, w2e_v, acc_sum, acc_max, scale_v, wsem,
          rsem, lsem, psem, *, inv_hw):
    n_a, n_r, n_c, n_w = xbuf.shape
    n_steps = n_c // _RK
    c_early = n_c - _RK
    r_late = n_r - _NLATE

    def issue_row(r, steps):
        sem = rsem.at[r % _DEPTH]
        for s in range(steps):
            for prio, (a0, na) in enumerate(((0, _SPLIT), (_SPLIT, n_a - _SPLIT))):
                sl = (pl.ds(a0, na), pl.ds(r, 1), pl.ds(s * _RK, _RK))
                pltpu.make_async_copy(
                    x_hbm.at[sl], xbuf.at[sl], sem).start(priority=prio)

    def wait_row(r, nch):
        sl = (slice(None), pl.ds(r, 1), pl.ds(0, nch))
        pltpu.make_async_copy(
            x_hbm.at[sl], xbuf.at[sl], rsem.at[r % _DEPTH]).wait()

    def issue_late():
        for i, (r0, nr) in enumerate(_LATE_GROUPS):
            for r in range(r_late + r0, r_late + r0 + nr):
                sl = (slice(None), pl.ds(r, 1), pl.ds(c_early, _RK))
                pltpu.make_async_copy(
                    x_hbm.at[sl], xbuf.at[sl], lsem.at[i]).start(priority=1)

    def wait_late(i):
        r0, nr = _LATE_GROUPS[i]
        sl = (slice(None), pl.ds(r_late + r0, nr), pl.ds(c_early, _RK))
        pltpu.make_async_copy(x_hbm.at[sl], xbuf.at[sl], lsem.at[i]).wait()

    w1cp = pltpu.make_async_copy(w1t_hbm, w1t_v, psem.at[0])
    w2cp = pltpu.make_async_copy(w2_hbm, w2_v, psem.at[1])

    issue_row(0, n_steps)
    w1cp.start()
    w2cp.start()

    def prologue(r, carry):
        issue_row(r, n_steps)
        return carry

    lax.fori_loop(1, _DEPTH, prologue, 0)

    acc_sum[...] = jnp.zeros(acc_sum.shape, _F32)
    acc_max[...] = jnp.full(acc_max.shape, -jnp.inf, _F32)

    w1cp.wait()
    w2cp.wait()
    zpad = jnp.zeros((64 - w1t_v.shape[0], n_c), _F32)
    w1t = w1t_v[...].astype(_F32)
    w1e_v[...] = jnp.concatenate([w1t, zpad, w1t, zpad], axis=0).T
    w2 = w2_v[...].astype(_F32)
    w2e_v[...] = jnp.concatenate([w2, zpad, w2, zpad], axis=0).T

    def accum_vals(r, c0, cg, s, m):
        for a in range(n_a):
            v = xbuf[a, r, pl.ds(c0, cg), :].astype(_F32)
            s = s + v
            m = jnp.maximum(m, v)
        return s, m

    def accum_group(r, c0, cg):
        s, m = accum_vals(r, c0, cg, acc_sum[pl.ds(c0, cg), :],
                          acc_max[pl.ds(c0, cg), :])
        acc_sum[pl.ds(c0, cg), :] = s
        acc_max[pl.ds(c0, cg), :] = m

    def accum_row(r, nch):
        def group(g, carry):
            accum_group(r, pl.multiple_of(g * _CG, _CG), _CG)
            return carry

        lax.fori_loop(0, nch // _CG, group, 0)
        if nch % _CG:
            accum_group(r, (nch // _CG) * _CG, nch % _CG)

    def steady(r, carry):
        wait_row(r, n_c)
        issue_row(r + _DEPTH, n_steps)
        accum_row(r, n_c)
        return carry

    lax.fori_loop(0, r_late - _DEPTH, steady, 0)

    for r in range(r_late - _DEPTH, n_r - 1):
        nch = n_c if r < r_late else c_early
        wait_row(r, nch)
        if r + _DEPTH < n_r:
            issue_row(r + _DEPTH, n_steps - 1)
        if r + _DEPTH == n_r - 1:
            issue_late()
        accum_row(r, nch)

    def layer1_partial(s, m, c0):
        n = s.shape[0]
        gap = jnp.sum(s, axis=1, keepdims=True) * inv_hw
        gap = gap.astype(_BF16).astype(_F32)
        gmp = jnp.max(m, axis=1, keepdims=True)
        lane = lax.broadcasted_iota(jnp.int32, (n, 128), 1)
        p = jnp.where(lane < 64, gap, gmp) * w1e_v[c0:c0 + n, :]
        return jnp.sum(p.reshape(n // 8, 8, 128), axis=0)

    wait_row(n_r - 1, c_early)
    q = jnp.zeros((8, 128), _F32)
    for c0 in range(0, c_early, _RK):
        s, m = accum_vals(n_r - 1, c0, _RK, acc_sum[c0:c0 + _RK, :],
                          acc_max[c0:c0 + _RK, :])
        q = q + layer1_partial(s, m, c0)

    s = acc_sum[c_early:n_c, :]
    m = acc_max[c_early:n_c, :]
    for i, (r0, nr) in enumerate(_LATE_GROUPS):
        wait_late(i)
        for r in range(r_late + r0, r_late + r0 + nr):
            s, m = accum_vals(r, c_early, _RK, s, m)

    q = q + layer1_partial(s, m, c_early)
    q = q + pltpu.roll(q, 4, 0)
    q = q + pltpu.roll(q, 2, 0)
    q = q + pltpu.roll(q, 1, 0)
    hid = jnp.maximum(q.astype(_BF16).astype(_F32), 0.0)
    prod = w2e_v[...].reshape(n_c // 8, 8, 128) * hid[None]
    z = jnp.sum(prod.reshape(n_c, 128), axis=1, keepdims=True)
    z = jnp.broadcast_to(z, (n_c, 128))

    def gate(logits):
        return jax.nn.sigmoid(logits).astype(_BF16).astype(_F32)

    n_head = sum(n for _, n in _HEAD)
    scale_v[0:n_head, :] = gate(z[0:n_head])
    scale_v[n_head:n_c, :] = z[n_head:n_c]

    def scale_and_store(r, c0, cg):
        s128 = scale_v[pl.ds(c0, cg), :]
        sc = jnp.concatenate([s128, s128[:, :n_w - 128]], axis=1)
        for a in range(n_a):
            v = xbuf[a, r, pl.ds(c0, cg), :].astype(_F32)
            xbuf[a, r, pl.ds(c0, cg), :] = (v * sc).astype(_BF16)
        sl = (slice(None), pl.ds(r, 1), pl.ds(c0, cg))
        pltpu.make_async_copy(xbuf.at[sl], o_hbm.at[sl], wsem.at[0]).start()

    for c0, n in _HEAD:
        scale_and_store(0, c0, n)

    def first_row(t, carry):
        c0 = pl.multiple_of(t * _WK, _WK)
        scale_v[pl.ds(c0, _WK), :] = gate(scale_v[pl.ds(c0, _WK), :])
        scale_and_store(0, c0, _WK)
        return carry

    lax.fori_loop(n_head // _WK, n_c // _WK, first_row, 0)

    def other_rows(r, carry):
        def chunk(t, c2):
            scale_and_store(r, pl.multiple_of(t * _WK, _WK), _WK)
            return c2

        return lax.fori_loop(0, n_c // _WK, chunk, carry)

    lax.fori_loop(1, n_r, other_rows, 0)


def _kernel(x_hbm, w1t_hbm, w2_hbm, o_hbm,
            xbuf, w1t_v, w2_v, w1e_v, w2e_v, acc_sum, acc_max, scale_v, wsem,
            *, inv_hw):
    pl.run_scoped(
        functools.partial(
            _body, x_hbm, w1t_hbm, w2_hbm, o_hbm, xbuf, w1t_v, w2_v, w1e_v,
            w2e_v, acc_sum, acc_max, scale_v, wsem, inv_hw=inv_hw),
        pltpu.SemaphoreType.DMA((_DEPTH,)),
        pltpu.SemaphoreType.DMA((len(_LATE_GROUPS),)),
        pltpu.SemaphoreType.DMA((2,)),
    )
    pltpu.make_async_copy(xbuf, o_hbm, wsem.at[0]).wait()


@jax.jit
def pallas_standalone__channel_attn_cbam__vision_kernel(
    x: jax.Array,
    w1: jax.Array,
    w2: jax.Array,
):
    B, H, W, C = x.shape
    r = w1.shape[1]
    assert B == 1 and H % _A == 0 and C % _WK == 0 and C % _CG == 0
    assert 128 < W <= 256 and r <= 64 and r % 8 == 0
    assert w1.shape == (C, r) and w2.shape == (r, C)
    R = H // _A
    assert R > _NLATE + _DEPTH

    x4 = jnp.transpose(x, (0, 1, 3, 2)).reshape(_A, R, C, W)
    w1t = w1.T

    out4 = pl.pallas_call(
        functools.partial(_kernel, inv_hw=1.0 / (H * W)),
        in_specs=[
            pl.BlockSpec(memory_space=pl.ANY),
            pl.BlockSpec(memory_space=pl.ANY),
            pl.BlockSpec(memory_space=pl.ANY),
        ],
        out_specs=pl.BlockSpec(memory_space=pl.ANY),
        out_shape=jax.ShapeDtypeStruct((_A, R, C, W), x.dtype),
        scratch_shapes=[
            pltpu.VMEM((_A, R, C, W), x.dtype),
            pltpu.VMEM((r, C), w1.dtype),
            pltpu.VMEM((r, C), w2.dtype),
            pltpu.VMEM((C, 128), _F32),
            pltpu.VMEM((C, 128), _F32),
            pltpu.VMEM((C, W), _F32),
            pltpu.VMEM((C, W), _F32),
            pltpu.VMEM((C, 128), _F32),
            pltpu.SemaphoreType.DMA((1,)),
        ],
        compiler_params=pltpu.CompilerParams(
            vmem_limit_bytes=64 * 1024 * 1024),
    )(x4, w1t, w2)

    return jnp.transpose(out4.reshape(B, H, C, W), (0, 1, 3, 2))
```

```python
import functools

import jax
import jax.numpy as jnp
from jax import lax
import jax.experimental.pallas as pl
import jax.experimental.pallas.tpu as pltpu


_A = 7
_PARTS = ((0, 0, 1), (1, 1, 2), (1, 3, 2), (1, 5, 2))
_RK = 32
_DEPTH = 4
_LC = 16
_NLATE = 6
_LATE_GROUPS = ((0, 3), (3, 2), (5, 1))
_CG = 32
_WK = 48
_WPARTS = ((0, 16), (16, 32))

_F32 = jnp.float32
_BF16 = jnp.bfloat16


def _body(x_hbm, w1t_hbm, w2_hbm, o_hbm,
          xbuf, w1t_v, w2_v, w1e_v, w2e_v, acc_sum, acc_max, scale_v, wsem,
          rsem, lsem, psem, *, inv_hw):
    n_a, n_r, n_c, n_w = xbuf.shape
    c_early = n_c - _LC
    r_late = n_r - _NLATE

    def issue_row(r, nch):
        sem = rsem.at[r % _DEPTH]
        for c0 in range(0, nch, _RK):
            for prio, a0, na in _PARTS:
                sl = (pl.ds(a0, na), pl.ds(r, 1), pl.ds(c0, min(_RK, nch - c0)))
                pltpu.make_async_copy(
                    x_hbm.at[sl], xbuf.at[sl], sem).start(priority=prio)

    def wait_row(r, nch):
        sl = (slice(None), pl.ds(r, 1), pl.ds(0, nch))
        pltpu.make_async_copy(
            x_hbm.at[sl], xbuf.at[sl], rsem.at[r % _DEPTH]).wait()

    def issue_late():
        for i, (r0, nr) in enumerate(_LATE_GROUPS):
            for r in range(r_late + r0, r_late + r0 + nr):
                sl = (slice(None), pl.ds(r, 1), pl.ds(c_early, _LC))
                pltpu.make_async_copy(
                    x_hbm.at[sl], xbuf.at[sl], lsem.at[i]).start(priority=1)

    def wait_late(i):
        r0, nr = _LATE_GROUPS[i]
        sl = (slice(None), pl.ds(r_late + r0, nr), pl.ds(c_early, _LC))
        pltpu.make_async_copy(x_hbm.at[sl], xbuf.at[sl], lsem.at[i]).wait()

    w1cp = pltpu.make_async_copy(w1t_hbm, w1t_v, psem.at[0])
    w2cp = pltpu.make_async_copy(w2_hbm, w2_v, psem.at[1])

    issue_row(0, n_c)
    w1cp.start()
    w2cp.start()

    def prologue(r, carry):
        issue_row(r, n_c)
        return carry

    lax.fori_loop(1, _DEPTH, prologue, 0)

    acc_sum[...] = jnp.zeros(acc_sum.shape, _F32)
    acc_max[...] = jnp.full(acc_max.shape, -jnp.inf, _F32)

    w1cp.wait()
    w2cp.wait()
    zpad = jnp.zeros((64 - w1t_v.shape[0], n_c), _F32)
    w1t = w1t_v[...].astype(_F32)
    w1e_v[...] = jnp.concatenate([w1t, zpad, w1t, zpad], axis=0).T
    w2 = w2_v[...].astype(_F32)
    w2e_v[...] = jnp.concatenate([w2, zpad, w2, zpad], axis=0).T

    def accum_vals(r, c0, cg, s, m):
        for a in range(n_a):
            v = xbuf[a, r, pl.ds(c0, cg), :].astype(_F32)
            s = s + v
            m = jnp.maximum(m, v)
        return s, m

    def accum_group(r, c0, cg):
        s, m = accum_vals(r, c0, cg, acc_sum[pl.ds(c0, cg), :],
                          acc_max[pl.ds(c0, cg), :])
        acc_sum[pl.ds(c0, cg), :] = s
        acc_max[pl.ds(c0, cg), :] = m

    def accum_row(r, nch):
        def group(g, carry):
            accum_group(r, pl.multiple_of(g * _CG, _CG), _CG)
            return carry

        lax.fori_loop(0, nch // _CG, group, 0)
        if nch % _CG:
            accum_group(r, (nch // _CG) * _CG, nch % _CG)

    def steady(r, carry):
        wait_row(r, n_c)
        issue_row(r + _DEPTH, n_c)
        accum_row(r, n_c)
        return carry

    lax.fori_loop(0, r_late - _DEPTH, steady, 0)

    for r in range(r_late - _DEPTH, n_r - 1):
        nch = n_c if r < r_late else c_early
        wait_row(r, nch)
        if r + _DEPTH < n_r:
            issue_row(r + _DEPTH, c_early)
        if r + _DEPTH == n_r - 1:
            issue_late()
        accum_row(r, nch)

    def layer1_partial(s, m, c0):
        n = s.shape[0]
        gap = jnp.sum(s, axis=1, keepdims=True) * inv_hw
        gap = gap.astype(_BF16).astype(_F32)
        gmp = jnp.max(m, axis=1, keepdims=True)
        lane = lax.broadcasted_iota(jnp.int32, (n, 128), 1)
        p = jnp.where(lane < 64, gap, gmp) * w1e_v[c0:c0 + n, :]
        return jnp.sum(p.reshape(n // 8, 8, 128), axis=0)

    wait_row(n_r - 1, c_early)
    q = jnp.zeros((8, 128), _F32)
    for c0 in range(0, c_early, _LC):
        s, m = accum_vals(n_r - 1, c0, _LC, acc_sum[c0:c0 + _LC, :],
                          acc_max[c0:c0 + _LC, :])
        q = q + layer1_partial(s, m, c0)

    s = acc_sum[c_early:n_c, :]
    m = acc_max[c_early:n_c, :]
    for i, (r0, nr) in enumerate(_LATE_GROUPS):
        wait_late(i)
        for r in range(r_late + r0, r_late + r0 + nr):
            s, m = accum_vals(r, c_early, _LC, s, m)

    q = q + layer1_partial(s, m, c_early)
    q = q + pltpu.roll(q, 4, 0)
    q = q + pltpu.roll(q, 2, 0)
    q = q + pltpu.roll(q, 1, 0)
    hid = jnp.maximum(q.astype(_BF16).astype(_F32), 0.0)
    prod = w2e_v[...].reshape(n_c // 8, 8, 128) * hid[None]
    z = jnp.sum(prod.reshape(n_c, 128), axis=1, keepdims=True)
    z = jnp.broadcast_to(z, (n_c, 128))

    def gate(logits):
        return jax.nn.sigmoid(logits).astype(_BF16).astype(_F32)

    scale_v[0:_WK, :] = gate(z[0:_WK])
    scale_v[_WK:n_c, :] = z[_WK:n_c]

    def scale_and_store(r, t):
        for off, cg in _WPARTS:
            c0 = t * _WK + off
            if not isinstance(c0, int):
                c0 = pl.multiple_of(c0, 16)
            s128 = scale_v[pl.ds(c0, cg), :]
            sc = jnp.concatenate([s128, s128[:, :n_w - 128]], axis=1)
            for a in range(n_a):
                v = xbuf[a, r, pl.ds(c0, cg), :].astype(_F32)
                xbuf[a, r, pl.ds(c0, cg), :] = (v * sc).astype(_BF16)
            sl = (slice(None), pl.ds(r, 1), pl.ds(c0, cg))
            pltpu.make_async_copy(xbuf.at[sl], o_hbm.at[sl], wsem.at[0]).start()

    scale_and_store(0, 0)

    def first_row(t, carry):
        c0 = pl.multiple_of(t * _WK, _WK)
        scale_v[pl.ds(c0, _WK), :] = gate(scale_v[pl.ds(c0, _WK), :])
        scale_and_store(0, t)
        return carry

    lax.fori_loop(1, n_c // _WK, first_row, 0)

    def other_rows(r, carry):
        def step(t, c2):
            scale_and_store(r, t)
            return c2

        return lax.fori_loop(0, n_c // _WK, step, carry)

    lax.fori_loop(1, n_r, other_rows, 0)


def _kernel(x_hbm, w1t_hbm, w2_hbm, o_hbm,
            xbuf, w1t_v, w2_v, w1e_v, w2e_v, acc_sum, acc_max, scale_v, wsem,
            *, inv_hw):
    pl.run_scoped(
        functools.partial(
            _body, x_hbm, w1t_hbm, w2_hbm, o_hbm, xbuf, w1t_v, w2_v, w1e_v,
            w2e_v, acc_sum, acc_max, scale_v, wsem, inv_hw=inv_hw),
        pltpu.SemaphoreType.DMA((_DEPTH,)),
        pltpu.SemaphoreType.DMA((len(_LATE_GROUPS),)),
        pltpu.SemaphoreType.DMA((2,)),
    )
    pltpu.make_async_copy(xbuf, o_hbm, wsem.at[0]).wait()


@jax.jit
def pallas_standalone__channel_attn_cbam__vision_kernel(
    x: jax.Array,
    w1: jax.Array,
    w2: jax.Array,
):
    B, H, W, C = x.shape
    r = w1.shape[1]
    assert B == 1 and H % _A == 0
    assert C % _WK == 0 and C % _CG == 0 and C % _RK == 0 and C % _LC == 0
    assert 128 < W <= 256 and r <= 64 and r % 8 == 0
    assert w1.shape == (C, r) and w2.shape == (r, C)
    R = H // _A
    assert R > _NLATE + _DEPTH

    x4 = jnp.transpose(x, (0, 1, 3, 2)).reshape(_A, R, C, W)
    w1t = w1.T

    out4 = pl.pallas_call(
        functools.partial(_kernel, inv_hw=1.0 / (H * W)),
        in_specs=[
            pl.BlockSpec(memory_space=pl.ANY),
            pl.BlockSpec(memory_space=pl.ANY),
            pl.BlockSpec(memory_space=pl.ANY),
        ],
        out_specs=pl.BlockSpec(memory_space=pl.ANY),
        out_shape=jax.ShapeDtypeStruct((_A, R, C, W), x.dtype),
        scratch_shapes=[
            pltpu.VMEM((_A, R, C, W), x.dtype),
            pltpu.VMEM((r, C), w1.dtype),
            pltpu.VMEM((r, C), w2.dtype),
            pltpu.VMEM((C, 128), _F32),
            pltpu.VMEM((C, 128), _F32),
            pltpu.VMEM((C, W), _F32),
            pltpu.VMEM((C, W), _F32),
            pltpu.VMEM((C, 128), _F32),
            pltpu.SemaphoreType.DMA((1,)),
        ],
        compiler_params=pltpu.CompilerParams(
            vmem_limit_bytes=64 * 1024 * 1024),
    )(x4, w1t, w2)

    return jnp.transpose(out4.reshape(B, H, C, W), (0, 1, 3, 2))
```
